```python
import os as _os
_os.environ.setdefault("JAX_PLATFORMS", "cpu")
import jax
import jax.numpy as jnp

def _softmax(x, axis=-1):
    return jax.nn.softmax(x, axis=axis)
def _gelu(x):
    return jax.nn.gelu(x, approximate=True)
def _silu(x):
    return jax.nn.silu(x)
def _sigmoid(x):
    return jax.nn.sigmoid(x)
def _layernorm(x, axis=-1, eps=1e-5):
    m = jnp.mean(x, axis=axis, keepdims=True)
    v = jnp.var(x, axis=axis, keepdims=True)
    return (x - m) / jnp.sqrt(v + eps)
def _scatter_add(tgt, idx, src, axis=0):
    return tgt.at[idx].add(src)
def _segment_sum(src, seg, n):
    return jax.ops.segment_sum(src, seg, n)
class _Rng:
    def __init__(self, key):
        self._k = key
    def _next(self):
        self._k, sub = jax.random.split(self._k)
        return sub
    def normal(self, shape):
        return jax.random.normal(self._next(), shape, dtype=jnp.bfloat16)
    def randint(self, lo, hi, shape):
        return jax.random.randint(self._next(), shape, lo, hi, dtype=jnp.int32)
    def uniform(self, shape, lo=0.0, hi=1.0):
        return jax.random.uniform(self._next(), shape, jnp.bfloat16, lo, hi)
    def permutation(self, n):
        return jax.random.permutation(self._next(), n)


kernel_name = 'standalone__gqa_softmax__decode'

def setup_inputs():
    _rng = _Rng(jax.random.key(int.from_bytes(__import__("os").urandom(4), "little")))
    _w = (lambda a: (lambda t: t.astype(jnp.bfloat16) if jnp.issubdtype(t.dtype, jnp.floating) else t)(jnp.asarray(a)))
    B, Hq, Hkv, Sq, Sk, D = 2, 32, 32, 1, 8192, 128
    return {
        "q": _w((lambda *s: _rng.normal(s) * 0.8)(B, Hq, Sq, D)),
        "k": _w((lambda *s: _rng.normal(s) * 0.8)(B, Hkv, Sk, D)),
        "v": _w((lambda *s: _rng.normal(s) * 0.05)(B, Hkv, Sk, D)),
    }

def reference(q, k, v):
    B, Hq, Sq, D = q.shape
    Hkv = k.shape[1]
    rep = Hq // Hkv
    k = jnp.repeat(k, rep, axis=1)
    v = jnp.repeat(v, rep, axis=1)
    scale = D ** -0.5
    scores = jnp.einsum("bhqd,bhkd->bhqk", q, k) * scale
    p = _softmax(scores, axis=-1)
    return jnp.einsum("bhqk,bhkd->bhqd", p, v)
```

```python
import jax
import jax.numpy as jnp
import jax.experimental.pallas as pl
import jax.experimental.pallas.tpu as pltpu

U = 2048
G = 8
CR = 16
BR = 256
NBUF = 6


@jax.jit
def pallas_standalone__gqa_softmax__decode_kernel(
    q: jax.Array,
    k: jax.Array,
    v: jax.Array,
):
    B, H, Sq, D = q.shape
    Hkv, Sk = k.shape[1], k.shape[2]
    assert Sq == 1 and H == Hkv
    BH = B * H
    scale = D ** -0.5
    upH = Sk // U
    hpg = G // upH
    NU = BH * upH
    ngroups = NU // G
    nper = U // BR
    nsteps = ngroups * nper
    nsub = BR // CR
    q2 = q.reshape(BH, D)
    k3 = k.reshape(NU, U, D)
    v3 = v.reshape(NU, U, D)

    def kern(q_hbm, k_hbm, v_hbm, o_ref, kbuf, vbuf, sem, qsem, qb, qf, of):
        def start_step(i, slot):
            g = i // nper
            j = i % nper
            for t in range(nsub):
                r = pl.multiple_of(j * BR + t * CR, CR)
                pltpu.make_async_copy(
                    k_hbm.at[pl.ds(g * G, G), pl.ds(r, CR)],
                    kbuf.at[slot, :, pl.ds(t * CR, CR)],
                    sem.at[0, slot]).start(priority=0)
                pltpu.make_async_copy(
                    v_hbm.at[pl.ds(g * G, G), pl.ds(r, CR)],
                    vbuf.at[slot, :, pl.ds(t * CR, CR)],
                    sem.at[1, slot]).start(priority=1)

        def wait_step(slot):
            pltpu.make_async_copy(kbuf.at[slot], kbuf.at[slot], sem.at[0, slot]).wait()
            pltpu.make_async_copy(vbuf.at[slot], vbuf.at[slot], sem.at[1, slot]).wait()

        qcp = pltpu.make_async_copy(q_hbm, qb, qsem.at[0])
        qcp.start()
        for b in range(NBUF - 1):
            start_step(b, b)
        qcp.wait()
        qf[...] = qb[...].astype(jnp.float32)

        def load(buf, slot, a):
            return buf[slot, a * upH:(a + 1) * upH].reshape(upH * BR, D)

        def group(g, c):
            qs = [jnp.broadcast_to(qf[pl.ds(g * hpg + a, 1), :], (8, D)).astype(k_hbm.dtype)
                  for a in range(hpg)]

            def step(j, st):
                i = g * nper + j
                slot = i % NBUF
                wait_step(slot)

                @pl.when(i + NBUF - 1 < nsteps)
                def _():
                    start_step(i + NBUF - 1, (i + NBUF - 1) % NBUF)

                new = []
                for a in range(hpg):
                    m, l, acc = st[a]
                    s = jax.lax.dot_general(
                        qs[a], load(kbuf, slot, a), (((1,), (1,)), ((), ())),
                        preferred_element_type=jnp.float32) * scale
                    mn = jnp.maximum(m, jnp.max(s, axis=-1, keepdims=True))
                    alpha = jnp.exp(m - mn)
                    p = jnp.exp(s - mn)
                    l = alpha * l + jnp.sum(p, axis=-1, keepdims=True)
                    acc = alpha * acc + jnp.dot(
                        p.astype(v_hbm.dtype), load(vbuf, slot, a),
                        preferred_element_type=jnp.float32)
                    new.append((mn, l, acc))
                return tuple(new)

            init = tuple(
                (jnp.full((8, 1), -jnp.inf, jnp.float32),
                 jnp.zeros((8, 1), jnp.float32),
                 jnp.zeros((8, D), jnp.float32)) for _ in range(hpg))
            st = jax.lax.fori_loop(0, nper, step, init)
            for a in range(hpg):
                _, l, acc = st[a]
                of[pl.ds(g * hpg + a, 1), :] = (acc / l)[0:1]
            return c

        jax.lax.fori_loop(0, ngroups, group, 0)
        o_ref[...] = of[...].astype(o_ref.dtype)

    bshape = (NBUF, G, BR, D)
    out = pl.pallas_call(
        kern,
        in_specs=[pl.BlockSpec(memory_space=pl.ANY)] * 3,
        out_specs=pl.BlockSpec(memory_space=pltpu.VMEM),
        out_shape=jax.ShapeDtypeStruct((BH, D), q.dtype),
        scratch_shapes=[
            pltpu.VMEM(bshape, k.dtype), pltpu.VMEM(bshape, v.dtype),
            pltpu.SemaphoreType.DMA((2, NBUF)), pltpu.SemaphoreType.DMA((1,)),
            pltpu.VMEM((BH, D), q.dtype), pltpu.VMEM((BH, D), jnp.float32),
            pltpu.VMEM((BH, D), jnp.float32)],
        compiler_params=pltpu.CompilerParams(vmem_limit_bytes=64 * 1024 * 1024),
    )(q2, k3, v3)
    return out.reshape(B, H, Sq, D)
```

```python
import jax
import jax.numpy as jnp
import jax.experimental.pallas as pl
import jax.experimental.pallas.tpu as pltpu

U = 2048
G = 16
CR = 8
BR = 128
NBUF = 4
H0 = 1


@jax.jit
def pallas_standalone__gqa_softmax__decode_kernel(
    q: jax.Array,
    k: jax.Array,
    v: jax.Array,
):
    B, H, Sq, D = q.shape
    Hkv, Sk = k.shape[1], k.shape[2]
    assert Sq == 1 and H == Hkv
    BH = B * H
    scale = D ** -0.5
    upH = Sk // U
    hpg = G // upH
    NU = BH * upH
    ngroups = NU // G
    nper = U // BR
    nsteps = ngroups * nper
    assert upH == 4 and hpg == 4 and H0 == 1
    q2 = q.reshape(BH, D)
    k3 = k.reshape(NU, U, D)
    v3 = v.reshape(NU, U, D)

    def gidx(o):
        return (o + ngroups - 1) % ngroups

    def kern(q_hbm, k_hbm, v_hbm, o_ref, kbuf, vbuf, sem, qsem, qb, qf, of):
        def pair(u, nu, r, nr, slot, s, t):
            pltpu.make_async_copy(
                k_hbm.at[pl.ds(u, nu), pl.ds(r, nr)],
                kbuf.at[slot, pl.ds(s, nu), pl.ds(t, nr)],
                sem.at[0, slot]).start(priority=0)
            pltpu.make_async_copy(
                v_hbm.at[pl.ds(u, nu), pl.ds(r, nr)],
                vbuf.at[slot, pl.ds(s, nu), pl.ds(t, nr)],
                sem.at[1, slot]).start(priority=1)

        def start_normal(o, j, slot):
            u = H0 * upH + gidx(o) * G
            for t in range(0, BR, CR):
                pair(u, G, pl.multiple_of(j * BR + t, CR), CR, slot, 0, t)

        def start_wrap(j, slot):
            ua = NU - 3 * upH
            for t in range(0, BR, 32):
                r = pl.multiple_of(j * BR + t, 32)
                pair(ua, 8, r, 16, slot, 0, t)
                pair(ua + 8, 4, r, 32, slot, 8, t)
                pair(ua, 8, r + 16, 16, slot, 0, t + 16)
                pair(0, 4, r, 32, slot, 12, t)

        def start_step(i, slot):
            o = i // nper
            j = i % nper

            @pl.when(o == 0)
            def _():
                start_wrap(j, slot)

            @pl.when(o != 0)
            def _():
                start_normal(o, j, slot)

        def wait_k(slot):
            pltpu.make_async_copy(kbuf.at[slot], kbuf.at[slot], sem.at[0, slot]).wait()

        def wait_v(slot):
            pltpu.make_async_copy(vbuf.at[slot], vbuf.at[slot], sem.at[1, slot]).wait()

        qcp = pltpu.make_async_copy(q_hbm, qb, qsem.at[0])
        start_wrap(0, 0)
        qcp.start()

        def prologue(b, c):
            start_wrap(b, b)
            return c

        jax.lax.fori_loop(1, NBUF - 1, prologue, 0)
        qcp.wait()
        qf[...] = qb[...].astype(jnp.float32)

        def load(buf, slot, a):
            return buf[slot, a * upH:(a + 1) * upH].reshape(upH * BR, D)

        def group(o, c):
            heads = [(H0 + gidx(o) * hpg + a) % BH for a in range(hpg)]
            qs = [jnp.broadcast_to(qf[pl.ds(heads[a], 1), :], (8, D)).astype(k_hbm.dtype)
                  for a in range(hpg)]

            def step(j, st):
                i = o * nper + j
                slot = i % NBUF

                @pl.when(i + NBUF - 1 < nsteps)
                def _():
                    start_step(i + NBUF - 1, (i + NBUF - 1) % NBUF)

                wait_k(slot)
                mid = []
                for a in range(hpg):
                    m, l, acc = st[a]
                    s = jax.lax.dot_general(
                        qs[a], load(kbuf, slot, a), (((1,), (1,)), ((), ())),
                        preferred_element_type=jnp.float32) * scale
                    mn = jnp.maximum(m, jnp.max(s, axis=-1, keepdims=True))
                    alpha = jnp.exp(m - mn)
                    p = jnp.exp(s - mn)
                    l = alpha * l + jnp.sum(p, axis=-1, keepdims=True)
                    mid.append((mn, l, alpha * acc, p.astype(v_hbm.dtype)))
                wait_v(slot)
                new = []
                for a in range(hpg):
                    mn, l, acc, p = mid[a]
                    acc = acc + jnp.dot(p, load(vbuf, slot, a),
                                        preferred_element_type=jnp.float32)
                    new.append((mn, l, acc))
                return tuple(new)

            init = tuple(
                (jnp.full((8, 1), -jnp.inf, jnp.float32),
                 jnp.zeros((8, 1), jnp.float32),
                 jnp.zeros((8, D), jnp.float32)) for _ in range(hpg))
            st = jax.lax.fori_loop(0, nper, step, init)
            for a in range(hpg):
                _, l, acc = st[a]
                of[pl.ds(heads[a], 1), :] = (acc / l)[0:1]
            return c

        jax.lax.fori_loop(0, ngroups, group, 0)
        o_ref[...] = of[...].astype(o_ref.dtype)

    bshape = (NBUF, G, BR, D)
    out = pl.pallas_call(
        kern,
        in_specs=[pl.BlockSpec(memory_space=pl.ANY)] * 3,
        out_specs=pl.BlockSpec(memory_space=pltpu.VMEM),
        out_shape=jax.ShapeDtypeStruct((BH, D), q.dtype),
        scratch_shapes=[
            pltpu.VMEM(bshape, k.dtype), pltpu.VMEM(bshape, v.dtype),
            pltpu.SemaphoreType.DMA((2, NBUF)), pltpu.SemaphoreType.DMA((1,)),
            pltpu.VMEM((BH, D), q.dtype), pltpu.VMEM((BH, D), jnp.float32),
            pltpu.VMEM((BH, D), jnp.float32)],
        compiler_params=pltpu.CompilerParams(disable_bounds_checks=True),
    )(q2, k3, v3)
    return out.reshape(B, H, Sq, D)
```

```python
import jax
import jax.numpy as jnp
import jax.experimental.pallas as pl
import jax.experimental.pallas.tpu as pltpu

U = 2048
G = 16
CR = 8
BR = 128
NBUF = 4
TAIL = 32
NP1 = 14


@jax.jit
def pallas_standalone__gqa_softmax__decode_kernel(
    q: jax.Array,
    k: jax.Array,
    v: jax.Array,
):
    B, H, Sq, D = q.shape
    Hkv, Sk = k.shape[1], k.shape[2]
    assert Sq == 1 and H == Hkv
    BH = B * H
    scale = D ** -0.5
    upH = Sk // U
    hpg = G // upH
    NU = BH * upH
    ngroups = NU // G
    nper = U // BR
    nsteps = ngroups * nper
    last = nsteps - 1
    sp = BR - TAIL
    assert upH == 4 and hpg == 4 and BH % 16 == 0
    q2 = q.reshape(BH, D)
    k3 = k.reshape(NU, U, D)
    v3 = v.reshape(NU, U, D)
    f32 = jnp.float32

    def gidx(o):
        return (o + ngroups - 1) % ngroups

    def kern(q_hbm, k_hbm, v_hbm, o_hbm, kbuf, vbuf, sem, xsem, qb, qf, of, ob):
        def pair(u, nu, r, nr, slot, s, t, pk=0, vsem=None):
            pltpu.make_async_copy(
                k_hbm.at[pl.ds(u, nu), pl.ds(r, nr)],
                kbuf.at[slot, pl.ds(s, nu), pl.ds(t, nr)],
                sem.at[0, slot]).start(priority=pk)
            pltpu.make_async_copy(
                v_hbm.at[pl.ds(u, nu), pl.ds(r, nr)],
                vbuf.at[slot, pl.ds(s, nu), pl.ds(t, nr)],
                sem.at[1, slot] if vsem is None else vsem).start(priority=1)

        def start_normal(o, j, slot, is_last=False):
            u = upH + gidx(o) * G
            for t in range(0, BR, CR):
                pair(u, G, pl.multiple_of(j * BR + t, CR), CR, slot, 0, t,
                     vsem=xsem.at[1] if (is_last and t >= sp) else None)

        def start_wrap(j, slot, first=False):
            ua = NU - 3 * upH
            n = 0
            for t in range(0, BR, CR):
                n += 1
                pair(ua, 3 * upH, pl.multiple_of(j * BR + t, CR), CR, slot, 0, t,
                     pk=1 if (first and n <= NP1) else 0)
                if t % 32 == CR:
                    n += 1
                    pair(0, upH, pl.multiple_of(j * BR + t - CR, 32), 32, slot,
                         3 * upH, t - CR, pk=1 if (first and n <= NP1) else 0)

        def start_step(i, slot):
            o = i // nper
            j = i % nper

            @pl.when(o == 0)
            def _():
                start_wrap(j, slot)

            @pl.when(jnp.logical_and(o != 0, i < last))
            def _():
                start_normal(o, j, slot)

            @pl.when(i == last)
            def _():
                start_normal(ngroups - 1, nper - 1, last % NBUF, is_last=True)

        def wait_all(ref, s):
            pltpu.make_async_copy(ref, ref, s).wait()

        qcp = pltpu.make_async_copy(q_hbm, qb, xsem.at[0])
        start_wrap(0, 0, first=True)
        qcp.start()

        def prologue(b, c):
            start_wrap(b, b)
            return c

        jax.lax.fori_loop(1, NBUF - 1, prologue, 0)
        qcp.wait()
        q32 = qb[...].astype(f32)
        qf[0:BH, :] = q32
        qf[BH:BH + 8, :] = q32[0:8]

        def load(buf, slot, a, r0, r1):
            return buf[slot, a * upH:(a + 1) * upH, r0:r1].reshape(upH * (r1 - r0), D)

        def pick(xs):
            row = jax.lax.broadcasted_iota(jnp.int32, xs[0].shape, 0)
            r = xs[0]
            for a in range(1, hpg):
                r = jnp.where(row == a + 1, xs[a], r)
            return r

        def qk(i, m, l):
            first = (i % nper) == 0
            slot = i % NBUF
            q8 = qf[pl.ds(gidx(i // nper) * hpg, 8), :].astype(k_hbm.dtype)
            m = jnp.where(first, -jnp.inf, m)
            l = jnp.where(first, 0.0, l)
            wait_all(kbuf.at[slot], sem.at[0, slot])
            s0, s1 = [
                pick([jax.lax.dot_general(
                    q8, load(kbuf, slot, a, r0, r1), (((1,), (1,)), ((), ())),
                    preferred_element_type=f32) for a in range(hpg)]) * scale
                for r0, r1 in ((0, sp), (sp, BR))]
            mn = jnp.maximum(m, jnp.maximum(jnp.max(s0, axis=-1, keepdims=True),
                                            jnp.max(s1, axis=-1, keepdims=True)))
            alpha = jnp.exp(m - mn)
            p0 = jnp.exp(s0 - mn)
            p1 = jnp.exp(s1 - mn)
            l = (alpha * l + jnp.sum(p0, axis=-1, keepdims=True)
                 + jnp.sum(p1, axis=-1, keepdims=True))
            return mn, l, alpha, p0.astype(v_hbm.dtype), p1.astype(v_hbm.dtype)

        def pv(p, slot, r0, r1):
            return pick([jnp.dot(p, load(vbuf, slot, a, r0, r1),
                                 preferred_element_type=f32) for a in range(hpg)])

        st0 = qk(0, jnp.zeros((8, 1), f32), jnp.zeros((8, 1), f32))

        def step(i, carry):
            m, l, alpha, p0, p1, acc = carry
            slot = i % NBUF

            @pl.when(i + NBUF - 1 < nsteps)
            def _():
                start_step(i + NBUF - 1, (i + NBUF - 1) % NBUF)

            nxt = qk(i + 1, m, l)
            acc = alpha * jnp.where((i % nper) == 0, 0.0, acc)
            wait_all(vbuf.at[slot], sem.at[1, slot])
            acc = acc + pv(p0, slot, 0, sp) + pv(p1, slot, sp, BR)

            @pl.when((i % nper) == nper - 1)
            def _():
                of[pl.ds(gidx(i // nper) * hpg + 1, hpg), :] = (acc / l)[1:1 + hpg]

            return nxt + (acc,)

        _, l, alpha, p0, p1, acc = jax.lax.fori_loop(
            0, last, step, st0 + (jnp.zeros((8, D), f32),))

        slot = last % NBUF
        of[0:1, :] = of[BH:BH + 1, :]
        ob[0:BH - 16, :] = of[0:BH - 16, :].astype(ob.dtype)
        c0 = pltpu.make_async_copy(
            ob.at[pl.ds(0, BH - 16)], o_hbm.at[pl.ds(0, BH - 16)], xsem.at[0])
        c0.start()
        row = jax.lax.broadcasted_iota(jnp.int32, (8, D), 0)
        mine = jnp.logical_and(row >= 1, row <= hpg)
        rl = 1.0 / l
        t0 = of[BH - 16:BH - 8, :]
        of[BH - 7:BH - 3, :] = jnp.zeros((hpg, D), f32)
        t1 = of[BH - 8:BH, :]
        wait_all(vbuf.at[slot, :, pl.ds(0, sp)], sem.at[1, slot])
        acc = alpha * acc + pv(p0, slot, 0, sp)
        wait_all(vbuf.at[slot, :, pl.ds(sp, TAIL)], xsem.at[1])
        acc = acc + pv(p1, slot, sp, BR)
        t1 = jnp.where(mine, acc * rl, t1)
        ob[BH - 16:BH, :] = jnp.concatenate([t0, t1], axis=0).astype(ob.dtype)
        c1 = pltpu.make_async_copy(
            ob.at[pl.ds(BH - 16, 16)], o_hbm.at[pl.ds(BH - 16, 16)], xsem.at[1])
        c1.start()
        c0.wait()
        c1.wait()

    bshape = (NBUF, G, BR, D)
    out = pl.pallas_call(
        kern,
        in_specs=[pl.BlockSpec(memory_space=pl.ANY)] * 3,
        out_specs=pl.BlockSpec(memory_space=pl.ANY),
        out_shape=jax.ShapeDtypeStruct((BH, D), q.dtype),
        scratch_shapes=[
            pltpu.VMEM(bshape, k.dtype), pltpu.VMEM(bshape, v.dtype),
            pltpu.SemaphoreType.DMA((2, NBUF)), pltpu.SemaphoreType.DMA((2,)),
            pltpu.VMEM((BH, D), q.dtype), pltpu.VMEM((BH + 8, D), f32),
            pltpu.VMEM((BH + 8, D), f32), pltpu.VMEM((BH, D), q.dtype)],
        compiler_params=pltpu.CompilerParams(
            disable_bounds_checks=True, disable_semaphore_checks=True),
    )(q2, k3, v3)
    return out.reshape(B, H, Sq, D)
```

```python
import jax
import jax.numpy as jnp
import jax.experimental.pallas as pl
import jax.experimental.pallas.tpu as pltpu

U = 2048
G = 16
CR = 8
BR = 128
LAG = 26
AHEAD = 2
TAIL = 32
ORDER = (15, 12, 1, 2, 13, 14, 3, 0, 9, 10, 7, 4, 11, 8, 5, 6)


@jax.jit
def pallas_standalone__gqa_softmax__decode_kernel(
    q: jax.Array,
    k: jax.Array,
    v: jax.Array,
):
    B, H, Sq, D = q.shape
    Hkv, Sk = k.shape[1], k.shape[2]
    BH = B * H
    scale = D ** -0.5
    f32 = jnp.float32
    ND = BR // CR
    upH = Sk // U
    hpg = G // upH
    NU = BH * upH
    ng = NU // G
    nper = U // BR
    assert Sq == 1 and H == Hkv and D == 128
    assert upH == 4 and hpg == 4 and ng == 16 and nper == 16
    assert sorted(ORDER) == list(range(ng))
    assert ORDER[0] == ng - 1 and ORDER[-1] % 2 == 0 and ND < LAG < 2 * ND
    sp = BR - TAIL
    half = nper // 2
    S1 = half + (ng - 1) * nper
    NS = S1 + half
    b0 = LAG - ND
    packed = [sum(ORDER[4 * w + i] << (4 * i) for i in range(4)) for w in range(4)]

    def grp(p):
        w = jnp.where(p < 8, jnp.where(p < 4, packed[0], packed[1]),
                      jnp.where(p < 12, packed[2], packed[3]))
        return (w >> (4 * (p % 4))) & 15

    def hint(x, n):
        return x if isinstance(x, int) else pl.multiple_of(x, n)

    def kern(q_hbm, k_hbm, v_hbm, o_hbm, kring, vring, pace, ksem, vsem, xsem,
             sc, qb, qf, of, ob, wb):
        def cp(ref, ring, sem, u, s, nu, r, nr, prio):
            r = hint(r, nr)
            pltpu.make_async_copy(
                ref.at[pl.ds(u, nu), pl.ds(r, nr)],
                ring.at[pl.ds(s, nu), pl.ds(r, nr)], sem).start(priority=prio)

        def regular(ref, ring, sem, g, j, idx, prio):
            cp(ref, ring, sem, upH + g * G, 0, G, j * BR + idx * CR, CR, prio)

        def wrapped(ref, ring, sem, j, idx, prio):
            ua = NU - 3 * upH
            r = j * BR + (idx // 4) * 32
            if idx % 4 == 0:
                cp(ref, ring, sem, ua, 0, 8, r, 16, prio)
            elif idx % 4 == 1:
                cp(ref, ring, sem, ua + 8, 8, 4, r, 32, prio)
            elif idx % 4 == 2:
                cp(ref, ring, sem, ua, 0, 8, r + 16, 16, prio)
            else:
                cp(ref, ring, sem, 0, 12, 4, r, 32, prio)

        def first_k(s, t, prio):
            c = 2 * t + prio
            j = 2 * s + c // ND
            wrapped(k_hbm, kring, ksem.at[j], j, c % ND, prio)

        def mid_k(s, t, prio):
            j = (s - half) % nper
            regular(k_hbm, kring, ksem.at[j], grp(1 + (s - half) // nper), j, t, prio)

        def first_v(s, t, prio):
            wrapped(v_hbm, vring, vsem.at[s - half], s - half, t, prio)

        def mid_v(s, t, prio):
            j = (s - half) % nper
            regular(v_hbm, vring, vsem.at[j], grp((s - half) // nper), j, t, prio)

        def last_v(s, t, prio):
            c = 2 * t + prio
            j = 2 * (s - S1) + c // ND
            si = j
            if c // ND == 1 and (c % ND) * CR >= sp:
                si = jnp.where(j == nper - 1, nper, j)
            regular(v_hbm, vring, vsem.at[si], ORDER[-1], j, c % ND, prio)

        def pacer(s, t, prio):
            n = (s - NS) * ND + t
            pltpu.make_async_copy(
                k_hbm.at[pl.ds(upH + n, 1), pl.ds(0, CR)],
                pace.at[pl.ds(n, 1)], xsem.at[2]).start(priority=prio)

        def issue(s, smin, smax):
            for dl, ts in ((1, range(0, ND - b0)), (2, range(ND - b0, ND))):
                for lo, hi, e0, e1 in (
                        (0, half - dl, first_k, first_k),
                        (half - dl, half, first_k, first_v),
                        (half, half + nper - dl, mid_k, first_v),
                        (half + nper - dl, S1 - dl, mid_k, mid_v),
                        (S1 - dl, S1, mid_k, last_v),
                        (S1, NS - dl, last_v, last_v),
                        (NS - dl, NS, last_v, pacer)):
                    if max(lo, smin) >= min(hi, smax):
                        continue

                    def body(e0=e0, e1=e1, dl=dl, ts=ts):
                        for t in ts:
                            e0(s, t, 0)
                            e1(s + dl, (t + b0) % ND, 1)

                    if lo <= smin and smax <= hi:
                        body()
                    else:
                        pl.when(jnp.logical_and(s >= lo, s < hi))(body)

        def wait_all(ref, s):
            pltpu.make_async_copy(ref, ref, s).wait()

        def wait_k(j):
            wait_all(kring.at[:, pl.ds(hint(j * BR, BR), BR)], ksem.at[j])

        def wait_v(j):
            wait_all(vring.at[:, pl.ds(hint(j * BR, BR), BR)], vsem.at[j])

        for d in range(LAG):
            first_k(d // ND, d % ND, 1)
        qcp = pltpu.make_async_copy(q_hbm, qb, xsem.at[0])
        qcp.start()

        def prologue(s, c):
            issue(s, 0, AHEAD)
            return c

        jax.lax.fori_loop(0, AHEAD, prologue, 0)
        qcp.wait()
        q32 = qb[...].astype(f32)
        qf[0:BH, :] = q32
        qf[BH:BH + 8, :] = q32[0:8]

        def load(ring, j, a, r0, r1):
            x = ring[a * upH:(a + 1) * upH, pl.ds(hint(j * BR + r0, 32), r1 - r0)]
            return x.reshape(upH * (r1 - r0), D)

        def pick(xs):
            row = jax.lax.broadcasted_iota(jnp.int32, xs[0].shape, 0)
            r = xs[0]
            for a in range(1, hpg):
                r = jnp.where(row == a + 1, xs[a], r)
            return r

        def fold(x, op):
            r = x[:, 0:128]
            for c in range(1, x.shape[1] // 128):
                r = op(r, x[:, 128 * c:128 * (c + 1)])
            return r

        def qk(q8, j, mrun):
            s0, s1 = [
                pick([jax.lax.dot_general(
                    q8, load(kring, j, a, r0, r1), (((1,), (1,)), ((), ())),
                    preferred_element_type=f32) for a in range(hpg)]) * scale
                for r0, r1 in ((0, sp), (sp, BR))]
            sc[j, :, 0:upH * sp] = s0
            sc[j, :, upH * sp:upH * BR] = s1
            return jnp.maximum(
                mrun, jnp.maximum(fold(s0, jnp.maximum), fold(s1, jnp.maximum)))

        def probs(j, m):
            p = jnp.exp(sc[j] - m)
            return p, fold(p, jnp.add)

        def pv(p, j, r0, r1):
            pb = p[:, upH * r0:upH * r1].astype(v_hbm.dtype)
            return pick([jnp.dot(pb, load(vring, j, a, r0, r1),
                                 preferred_element_type=f32) for a in range(hpg)])

        def pv_full(p, j):
            return pv(p, j, 0, sp) + pv(p, j, sp, BR)

        def q_of(g):
            return qf[pl.ds(g * hpg, 8), :].astype(k_hbm.dtype)

        ninf = jnp.full((8, 128), -jnp.inf, f32)
        zero = jnp.zeros((8, 128), f32)

        q_first = q_of(ORDER[0])

        def it_first(c, mrun):
            issue(c + AHEAD, AHEAD, half + AHEAD)
            wait_k(2 * c)
            wait_k(2 * c + 1)
            return qk(q_first, 2 * c + 1, qk(q_first, 2 * c, mrun))

        mrun = jax.lax.fori_loop(0, half, it_first, ninf)

        def phase(p, mrun):
            m = jnp.max(mrun, axis=-1, keepdims=True)
            q8 = q_of(grp(p))

            def it(j, carry):
                mr, ls, acc = carry
                issue(half + (p - 1) * nper + j + AHEAD, half + AHEAD, S1 + AHEAD)
                pr, ps = probs(j, m)
                wait_k(j)
                wait_v(j)
                acc = acc + pv_full(pr, j)
                return qk(q8, j, mr), ls + ps, acc

            mr, ls, acc = jax.lax.fori_loop(0, nper, it, (ninf, zero, zero))
            res = acc / jnp.sum(ls, axis=-1, keepdims=True)
            of[pl.ds(grp(p - 1) * hpg + 1, hpg), :] = res[1:1 + hpg]
            return mr

        mrun = jax.lax.fori_loop(1, ng, phase, mrun)

        m = jnp.max(mrun, axis=-1, keepdims=True)
        r0 = ORDER[-1] * hpg
        t16 = (r0 // 16) * 16
        of[0:1, :] = of[BH:BH + 1, :]
        of[r0 + 1:r0 + 1 + hpg, :] = jnp.zeros((hpg, D), f32)
        ob[...] = of[0:BH, :].astype(ob.dtype)
        early = []
        for i, (a, n) in enumerate(((0, t16), (t16 + 16, BH - t16 - 16))):
            if n > 0:
                early.append(pltpu.make_async_copy(
                    ob.at[pl.ds(a, n)], o_hbm.at[pl.ds(a, n)], xsem.at[i]))
        for c in early:
            c.start()
        pt = jnp.exp(sc[nper - 1, :, upH * sp:upH * BR] - m).T
        for a in range(hpg):
            wb[a] = jnp.broadcast_to(pt[:, a + 1:a + 2], (upH * TAIL, D))

        def it_last(c, carry):
            ls, acc = carry

            @pl.when(S1 + c + AHEAD < NS)
            def _():
                issue(S1 + c + AHEAD, S1 + AHEAD, NS)

            pa, sa = probs(2 * c, m)
            pb, sb = probs(2 * c + 1, m)
            wait_v(2 * c)
            wait_v(2 * c + 1)
            return ls + sa + sb, acc + pv_full(pa, 2 * c) + pv_full(pb, 2 * c + 1)

        ls, acc = jax.lax.fori_loop(0, half - 1, it_last, (zero, zero))
        ja, jb = nper - 2, nper - 1
        pa, sa = probs(ja, m)
        pb, sb = probs(jb, m)
        rl = 1.0 / jnp.sum(ls + sa + sb, axis=-1, keepdims=True)
        row = jax.lax.broadcasted_iota(jnp.int32, (8, D), 0)
        mine = jnp.logical_and(row >= 1, row <= hpg)
        tiles = [of[t16:t16 + 8, :], of[t16 + 8:t16 + 16, :]]
        for c in early:
            c.wait()
        wait_v(ja)
        acc = acc + pv_full(pa, ja)
        wait_all(vring.at[:, pl.ds(jb * BR, sp)], vsem.at[jb])
        acc = acc + pv(pb, jb, 0, sp)
        wait_all(vring.at[:, pl.ds(jb * BR + sp, TAIL)], vsem.at[nper])
        acc = acc + pick([
            jnp.broadcast_to(
                jnp.sum(wb[a] * load(vring, jb, a, sp, BR).astype(f32),
                        axis=0, keepdims=True), (8, D)) for a in range(hpg)])
        w = (r0 - t16) // 8
        tiles[w] = jnp.where(mine, acc * rl, tiles[w])
        ob[t16:t16 + 16, :] = jnp.concatenate(tiles, axis=0).astype(ob.dtype)
        late = pltpu.make_async_copy(
            ob.at[pl.ds(t16, 16)], o_hbm.at[pl.ds(t16, 16)], xsem.at[0])
        late.start()
        wait_all(pace, xsem.at[2])
        late.wait()

    out = pl.pallas_call(
        kern,
        in_specs=[pl.BlockSpec(memory_space=pl.ANY)] * 3,
        out_specs=pl.BlockSpec(memory_space=pl.ANY),
        out_shape=jax.ShapeDtypeStruct((BH, D), q.dtype),
        scratch_shapes=[
            pltpu.VMEM((G, U, D), k.dtype),
            pltpu.VMEM((G, U, D), v.dtype),
            pltpu.VMEM((LAG, CR, D), k.dtype),
            pltpu.SemaphoreType.DMA((nper,)),
            pltpu.SemaphoreType.DMA((nper + 1,)),
            pltpu.SemaphoreType.DMA((3,)),
            pltpu.VMEM((nper, 8, upH * BR), f32),
            pltpu.VMEM((BH, D), q.dtype),
            pltpu.VMEM((BH + 8, D), f32),
            pltpu.VMEM((BH + 8, D), f32),
            pltpu.VMEM((BH, D), q.dtype),
            pltpu.VMEM((hpg, upH * TAIL, D), f32),
        ],
        compiler_params=pltpu.CompilerParams(
            vmem_limit_bytes=40 * 1024 * 1024,
            disable_bounds_checks=True, disable_semaphore_checks=True),
    )(q.reshape(BH, D), k.reshape(NU, U, D), v.reshape(NU, U, D))
    return out.reshape(B, H, Sq, D)
```

```python
import jax
import jax.numpy as jnp
import jax.experimental.pallas as pl
import jax.experimental.pallas.tpu as pltpu

U = 2048
G = 16
CR = 8
BR = 128
LAG = 26
AHEAD = 2
R1, R2 = 96, 120
ODD = (15, 1, 5, 7, 9, 11, 13, 3)
XOR = 7


@jax.jit
def pallas_standalone__gqa_softmax__decode_kernel(
    q: jax.Array,
    k: jax.Array,
    v: jax.Array,
):
    B, H, Sq, D = q.shape
    Hkv, Sk = k.shape[1], k.shape[2]
    BH = B * H
    scale = D ** -0.5
    f32 = jnp.float32
    ND = BR // CR
    upH = Sk // U
    hpg = G // upH
    NU = BH * upH
    ng = NU // G
    nper = U // BR
    npair = ng // 2
    assert Sq == 1 and H == Hkv and D == 128 and k.dtype == v.dtype
    assert upH == 4 and hpg == 4 and ng == 16 and nper == 16
    assert sorted(ODD) == list(range(1, ng, 2)) and XOR % 2 == 1
    assert ODD[0] == ng - 1 and ODD[-1] < 8 and ND < LAG < 2 * ND
    b0 = LAG - ND
    CA = upH * R1
    packed = sum(ODD[i] << (4 * i) for i in range(npair))
    both = jnp.logical_and

    def odd_group(n):
        return ODD[n] if isinstance(n, int) else (packed >> (4 * n)) & 15

    def hint(x, n):
        return x if isinstance(x, int) else pl.multiple_of(x, n)

    def kern(q_hbm, k_hbm, v_hbm, o_hbm, ring, pace, sem, xsem,
             sc, qb, qf, of, ob, wb):
        def cp(ref, th, si, u, s, nu, r):
            r = hint(r, CR)
            pltpu.make_async_copy(
                ref.at[pl.ds(u, nu), pl.ds(r, CR)],
                ring.at[th, pl.ds(s, nu), pl.ds(r, CR)],
                sem.at[si]).start(priority=th)

        def regular(ref):
            def emit1(n, j, t, th):
                g = odd_group(n) ^ (XOR * th)
                si = j
                if ref is v_hbm and t * CR >= R1:
                    si = jnp.where(both(n == npair - 1, j == nper - 1),
                                   nper + int(t * CR >= R2), j)
                cp(ref, th, si, upH + g * G, 0, G, j * BR + t * CR)
            return emit1

        def wrapped(ref):
            def emit1(n, j, t, th):
                cp(ref, th, j, NU - 3 * upH, 0, 3 * upH, j * BR + t * CR)
                cp(ref, th, j, 0, 3 * upH, upH, j * BR + t * CR)
            return emit1

        def pacer(n, j, t, th):
            i = j * ND + t
            pltpu.make_async_copy(
                k_hbm.at[pl.ds(upH + i, 1), pl.ds(0, CR)],
                pace.at[pl.ds(i, 1)], xsem.at[2]).start(priority=th)

        K, V = regular(k_hbm), regular(v_hbm)
        Kw, Vw = wrapped(k_hbm), wrapped(v_hbm)
        halves = ((1, range(0, ND - b0)), (2, range(ND - b0, ND)))

        def emit(cond, ts, e0, n0, j0, e1, n1, j1):
            def body():
                for t in ts:
                    e0(n0, j0, t, 0)
                    e1(n1, j1, (t + b0) % ND, 1)

            if cond is True:
                body()
            else:
                pl.when(cond)(body)

        def issue_in_k_phase(n, x):
            for dl, ts in halves:
                c1 = x < nper - dl
                c2 = both(x >= nper - dl, x < nper)
                c3 = x >= nper
                for c, k0, v0 in ((n == 0, Kw, Vw), (n != 0, K, V)):
                    emit(both(c, c1), ts, k0, n, x, K, n, x + dl)
                    emit(both(c, c2), ts, k0, n, x, V, n, x + dl - nper)
                    emit(both(c, c3), ts, v0, n, x - nper, V, n, x + dl - nper)

        def issue_in_v_phase(n, x):
            nn = jnp.minimum(n + 1, npair - 1)
            more = n != npair - 1
            for dl, ts in halves:
                c1 = x < nper - dl
                c2 = both(x >= nper - dl, x < nper)
                c3 = x >= nper
                y = x + dl - nper
                emit(both(n == 0, c1), ts, Vw, n, x, V, n, x + dl)
                emit(both(n != 0, c1), ts, V, n, x, V, n, x + dl)
                emit(both(n == 0, c2), ts, Vw, n, x, K, nn, y)
                emit(both(both(n != 0, more), c2), ts, V, n, x, K, nn, y)
                emit(both(n == npair - 1, c2), ts, V, n, x, pacer, nn, y)
                emit(both(more, c3), ts, K, nn, x - nper, K, nn, y)

        def wait_rows(r, nr, si):
            ref = ring.at[:, :, pl.ds(hint(r, CR), nr)]
            pltpu.make_async_copy(ref, ref, sem.at[si]).wait()

        for d in range(LAG):
            K(0, d // ND, d % ND, 1)
        qcp = pltpu.make_async_copy(q_hbm, qb, xsem.at[0])
        qcp.start()

        def prologue(s, c):
            for dl, ts in halves:
                emit(True, ts, Kw, 0, s, K, 0, s + dl)
            return c

        jax.lax.fori_loop(0, AHEAD, prologue, 0)
        of[...] = jnp.zeros(of.shape, f32)
        qcp.wait()
        qf[...] = qb[...].astype(f32).reshape(qf.shape)

        sub = [(5 + h) % 8 for h in range(8)]

        def load(j, h, r0, r1):
            u = (h % hpg) * upH
            x = ring[h // hpg, u:u + upH, pl.ds(hint(j * BR + r0, CR), r1 - r0)]
            return x.reshape(upH * (r1 - r0), D)

        def load_a(j, h):
            return load(j, h, 0, R1)

        def load_b(j, h):
            return jnp.concatenate([load(j, h, R1, R2), load(j, h, R2, BR)], axis=0)

        def pick(xs):
            rw = jax.lax.broadcasted_iota(jnp.int32, xs[0].shape, 0)
            r = xs[0]
            for h in range(1, 8):
                r = jnp.where(rw == sub[h], xs[h], r)
            return r

        def fold(x, op):
            r = x[:, 0:128]
            for c in range(1, x.shape[1] // 128):
                r = op(r, x[:, 128 * c:128 * (c + 1)])
            return r

        def scores(q8, j, ld):
            return pick([jax.lax.dot_general(
                q8, ld(j, h), (((1,), (1,)), ((), ())),
                preferred_element_type=f32) for h in range(8)]) * scale

        def probs(j, m):
            p = jnp.exp(sc[j] - m)
            return p.astype(v_hbm.dtype), fold(p, jnp.add)

        def pv(p, j, ld):
            return pick([jnp.dot(p, ld(j, h), preferred_element_type=f32)
                         for h in range(8)])

        row = jax.lax.broadcasted_iota(jnp.int32, (8, D), 0)
        row_masks = (row >= 5, row == 0, both(row >= 1, row <= 4))
        zero = jnp.zeros((8, 128), f32)

        def tiles_of(a):
            return (a - 1) // 2, ((a + 1) // 2) % (BH // 8), (a ^ XOR) // 2

        last_tiles = tiles_of(ODD[-1])
        o_lo, o_hi = min(last_tiles) * 8, max(last_tiles) * 8 + 8
        early = [
            pltpu.make_async_copy(ob.at[pl.ds(a, n)], o_hbm.at[pl.ds(a, n)], xsem.at[i])
            for i, (a, n) in enumerate(((0, o_lo), (o_hi, BH - o_hi))) if n > 0]

        def pair(n, carry):
            ts = tiles_of(odd_group(n))
            q8 = jnp.where(row_masks[0], qf[ts[0]],
                           jnp.where(row_masks[1], qf[ts[1]], qf[ts[2]]))
            q8 = q8.astype(k_hbm.dtype)
            last = n == npair - 1

            def k_step(j, mrun):
                issue_in_k_phase(n, j + AHEAD)
                wait_rows(j * BR, BR, j)
                s0 = scores(q8, j, load_a)
                s1 = scores(q8, j, load_b)
                sc[j, :, 0:CA] = s0
                sc[j, :, CA:] = s1
                return jnp.maximum(mrun, jnp.maximum(fold(s0, jnp.maximum), s1))

            mrun = jax.lax.fori_loop(
                0, nper, k_step, jnp.full((8, 128), -jnp.inf, f32))
            m = jnp.max(mrun, axis=-1, keepdims=True)

            def v_step(j, c):
                ls, acc = c
                issue_in_v_phase(n, j + AHEAD)

                @pl.when(both(last, j == 0))
                def _():
                    ob[...] = of[...].reshape(BH, D).astype(ob.dtype)
                    for cpy in early:
                        cpy.start()

                @pl.when(both(last, j == 1))
                def _():
                    pt = jnp.exp(sc[nper - 1, :, CA:] - m).T
                    for h in range(8):
                        wb[h] = jnp.broadcast_to(pt[:, sub[h]:sub[h] + 1], wb.shape[1:])

                p, ps = probs(j, m)
                wait_rows(j * BR, BR, j)
                return (ls + ps,
                        acc + pv(p[:, 0:CA], j, load_a) + pv(p[:, CA:], j, load_b))

            ls, acc = jax.lax.fori_loop(
                0, jnp.where(last, nper - 1, nper), v_step, (zero, zero))

            @pl.when(n != npair - 1)
            def _():
                res = acc / jnp.sum(ls, axis=-1, keepdims=True)
                for t, mask in zip(ts, row_masks):
                    of[t] = jnp.where(mask, res, of[t])

            return m, ls, acc

        m, ls, acc = jax.lax.fori_loop(
            0, npair, pair, (jnp.zeros((8, 1), f32), zero, zero))

        j = nper - 1
        p, ps = probs(j, m)
        rl = 1.0 / jnp.sum(ls + ps, axis=-1, keepdims=True)
        tiles = {t: of[t] for t in range(o_lo // 8, o_hi // 8)}
        for cpy in early:
            cpy.wait()
        wait_rows(j * BR, R1, j)
        acc = acc + pv(p[:, 0:CA], j, load_a)

        def pv_vpu(r0, r1):
            k0, n = upH * (r0 - R1), upH * (r1 - r0)
            return [jnp.sum((wb[h, k0:k0 + n] * load(j, h, r0, r1).astype(f32))
                            .reshape(n // 8, 8, D), axis=0) for h in range(8)]

        wait_rows(j * BR + R1, R2 - R1, nper)
        part = pv_vpu(R1, R2)
        wait_rows(j * BR + R2, BR - R2, nper + 1)
        acc = acc + pick([
            jnp.broadcast_to(jnp.sum(x + y, axis=0, keepdims=True), (8, D))
            for x, y in zip(part, pv_vpu(R2, BR))])
        res = acc * rl
        for t, mask in zip(last_tiles, row_masks):
            tiles[t] = jnp.where(mask, res, tiles[t])
        ob[o_lo:o_hi, :] = jnp.concatenate(
            [tiles[t] for t in sorted(tiles)], axis=0).astype(ob.dtype)
        late = pltpu.make_async_copy(
            ob.at[pl.ds(o_lo, o_hi - o_lo)], o_hbm.at[pl.ds(o_lo, o_hi - o_lo)],
            xsem.at[0])
        late.start()
        pltpu.make_async_copy(pace, pace, xsem.at[2]).wait()
        late.wait()

    out = pl.pallas_call(
        kern,
        in_specs=[pl.BlockSpec(memory_space=pl.ANY)] * 3,
        out_specs=pl.BlockSpec(memory_space=pl.ANY),
        out_shape=jax.ShapeDtypeStruct((BH, D), q.dtype),
        scratch_shapes=[
            pltpu.VMEM((2, G, U, D), k.dtype),
            pltpu.VMEM((LAG, CR, D), k.dtype),
            pltpu.SemaphoreType.DMA((nper + 2,)),
            pltpu.SemaphoreType.DMA((3,)),
            pltpu.VMEM((nper, 8, upH * BR), f32),
            pltpu.VMEM((BH, D), q.dtype),
            pltpu.VMEM((BH // 8, 8, D), f32),
            pltpu.VMEM((BH // 8, 8, D), f32),
            pltpu.VMEM((BH, D), q.dtype),
            pltpu.VMEM((8, upH * (BR - R1), D), f32),
        ],
        compiler_params=pltpu.CompilerParams(
            vmem_limit_bytes=40 * 1024 * 1024,
            disable_bounds_checks=True, disable_semaphore_checks=True),
    )(q.reshape(BH, D), k.reshape(NU, U, D), v.reshape(NU, U, D))
    return out.reshape(B, H, Sq, D)
```

```python
import jax
import jax.numpy as jnp
import jax.experimental.pallas as pl
import jax.experimental.pallas.tpu as pltpu

U = 2048
G = 16
CR = 8
BR = 128
LAG = 26
AHEAD = 2
R1, R2 = 96, 120
ODD = (15, 1, 5, 7, 9, 11, 13, 3)
XOR = 7


@jax.jit
def pallas_standalone__gqa_softmax__decode_kernel(
    q: jax.Array,
    k: jax.Array,
    v: jax.Array,
):
    B, H, Sq, D = q.shape
    Hkv, Sk = k.shape[1], k.shape[2]
    BH = B * H
    scale = D ** -0.5
    f32 = jnp.float32
    ND = BR // CR
    upH = Sk // U
    hpg = G // upH
    NU = BH * upH
    ng = NU // G
    nper = U // BR
    npair = ng // 2
    assert Sq == 1 and H == Hkv and D == 128
    assert upH == 4 and hpg == 4 and ng == 16 and nper == 16
    assert sorted(ODD) == list(range(1, ng, 2)) and XOR % 2 == 1
    assert ODD[0] == ng - 1 and ODD[-1] < 8 and ND < LAG < 2 * ND
    b0 = LAG - ND
    CA = upH * R1
    packed = sum(ODD[i] << (4 * i) for i in range(npair))
    both = jnp.logical_and

    def odd_group(n):
        return ODD[n] if isinstance(n, int) else (packed >> (4 * n)) & 15

    def hint(x, n):
        return x if isinstance(x, int) else pl.multiple_of(x, n)

    def kern(q_hbm, k_hbm, v_hbm, o_hbm, k0, k1, v0, v1, pace, sem, xsem,
             sc, qb, qf, of, ob, wb):
        kbufs, vbufs = (k0, k1), (v0, v1)

        def cp(ref, th, si, u, s, nu, r):
            r = hint(r, CR)
            buf = (kbufs if ref is k_hbm else vbufs)[th]
            pltpu.make_async_copy(
                ref.at[pl.ds(u, nu), pl.ds(r, CR)],
                buf.at[pl.ds(s, nu), pl.ds(r, CR)],
                sem.at[th, si]).start(priority=th)

        def regular(ref):
            def emit1(n, j, t, th):
                g = odd_group(n) ^ (XOR * th)
                si = j
                if ref is v_hbm and t * CR >= R1:
                    si = jnp.where(both(n == npair - 1, j == nper - 1),
                                   nper + int(t * CR >= R2), j)
                cp(ref, th, si, upH + g * G, 0, G, j * BR + t * CR)
            return emit1

        def wrapped(ref):
            def emit1(n, j, t, th):
                cp(ref, th, j, NU - 3 * upH, 0, 3 * upH, j * BR + t * CR)
                cp(ref, th, j, 0, 3 * upH, upH, j * BR + t * CR)
            return emit1

        def pacer(n, j, t, th):
            i = j * ND + t
            pltpu.make_async_copy(
                k_hbm.at[pl.ds(upH + i, 1), pl.ds(0, CR)],
                pace.at[pl.ds(i, 1)], xsem.at[2]).start(priority=th)

        K, V = regular(k_hbm), regular(v_hbm)
        Kw, Vw = wrapped(k_hbm), wrapped(v_hbm)
        halves = ((1, range(0, ND - b0)), (2, range(ND - b0, ND)))

        def emit(cond, ts, e0, n0, j0, e1, n1, j1):
            def body():
                for t in ts:
                    e0(n0, j0, t, 0)
                    e1(n1, j1, (t + b0) % ND, 1)

            if cond is True:
                body()
            else:
                pl.when(cond)(body)

        def issue_in_k_phase(n, x):
            for dl, ts in halves:
                c1 = x < nper - dl
                c2 = both(x >= nper - dl, x < nper)
                c3 = x >= nper
                for c, ek, ev in ((n == 0, Kw, Vw), (n != 0, K, V)):
                    emit(both(c, c1), ts, ek, n, x, K, n, x + dl)
                    emit(both(c, c2), ts, ek, n, x, V, n, x + dl - nper)
                    emit(both(c, c3), ts, ev, n, x - nper, V, n, x + dl - nper)

        def issue_in_v_phase(n, x):
            nn = jnp.minimum(n + 1, npair - 1)
            more = n != npair - 1
            for dl, ts in halves:
                c1 = x < nper - dl
                c2 = both(x >= nper - dl, x < nper)
                c3 = x >= nper
                y = x + dl - nper
                emit(both(n == 0, c1), ts, Vw, n, x, V, n, x + dl)
                emit(both(n != 0, c1), ts, V, n, x, V, n, x + dl)
                emit(both(n == 0, c2), ts, Vw, n, x, K, nn, y)
                emit(both(both(n != 0, more), c2), ts, V, n, x, K, nn, y)
                emit(both(n == npair - 1, c2), ts, V, n, x, pacer, nn, y)
                emit(both(more, c3), ts, K, nn, x - nper, K, nn, y)

        def fetch(bufs, r, nr, si):
            rows = pl.ds(hint(r, CR), nr)
            for th in range(2):
                ref = bufs[th].at[:, rows]
                pltpu.make_async_copy(ref, ref, sem.at[th, si]).wait()
            return [bufs[th][:, rows] for th in range(2)]

        for d in range(LAG):
            K(0, d // ND, d % ND, 1)
        qcp = pltpu.make_async_copy(q_hbm, qb, xsem.at[0])
        qcp.start()

        def prologue(s, c):
            for dl, ts in halves:
                emit(True, ts, Kw, 0, s, K, 0, s + dl)
            return c

        jax.lax.fori_loop(0, AHEAD, prologue, 0)
        of[...] = jnp.zeros(of.shape, f32)
        qcp.wait()
        qf[...] = qb[...].astype(f32).reshape(qf.shape)

        sub = [(5 + h) % 8 for h in range(8)]

        def part(xs, h, r0, r1):
            u = (h % hpg) * upH
            return xs[h // hpg][u:u + upH, r0:r1].reshape(upH * (r1 - r0), D)

        def part_a(xs, h):
            return part(xs, h, 0, R1)

        def part_b(xs, h):
            return jnp.concatenate([part(xs, h, R1, R2), part(xs, h, R2, BR)], axis=0)

        def pick(xs):
            rw = jax.lax.broadcasted_iota(jnp.int32, xs[0].shape, 0)
            r = xs[0]
            for h in range(1, 8):
                r = jnp.where(rw == sub[h], xs[h], r)
            return r

        def fold(x, op):
            r = x[:, 0:128]
            for c in range(1, x.shape[1] // 128):
                r = op(r, x[:, 128 * c:128 * (c + 1)])
            return r

        def scores(q8, xs, sel):
            return pick([jax.lax.dot_general(
                q8, sel(xs, h), (((1,), (1,)), ((), ())),
                preferred_element_type=f32) for h in range(8)]) * scale

        def probs(j, m):
            p = jnp.exp(sc[j] - m)
            return p.astype(v_hbm.dtype), fold(p, jnp.add)

        def pv(p, xs, sel):
            return pick([jnp.dot(p, sel(xs, h), preferred_element_type=f32)
                         for h in range(8)])

        row = jax.lax.broadcasted_iota(jnp.int32, (8, D), 0)
        row_masks = (row >= 5, row == 0, both(row >= 1, row <= 4))
        zero = jnp.zeros((8, 128), f32)

        def tiles_of(a):
            return (a - 1) // 2, ((a + 1) // 2) % (BH // 8), (a ^ XOR) // 2

        last_tiles = tiles_of(ODD[-1])
        o_lo, o_hi = min(last_tiles) * 8, max(last_tiles) * 8 + 8
        early = [
            pltpu.make_async_copy(ob.at[pl.ds(a, n)], o_hbm.at[pl.ds(a, n)], xsem.at[i])
            for i, (a, n) in enumerate(((0, o_lo), (o_hi, BH - o_hi))) if n > 0]

        def pair(n, carry):
            ts = tiles_of(odd_group(n))
            q8 = jnp.where(row_masks[0], qf[ts[0]],
                           jnp.where(row_masks[1], qf[ts[1]], qf[ts[2]]))
            q8 = q8.astype(k_hbm.dtype)
            last = n == npair - 1

            def k_step(j, mrun):
                issue_in_k_phase(n, j + AHEAD)
                xs = fetch(kbufs, j * BR, BR, j)
                s0 = scores(q8, xs, part_a)
                s1 = scores(q8, xs, part_b)
                sc[j, :, 0:CA] = s0
                sc[j, :, CA:] = s1
                return jnp.maximum(mrun, jnp.maximum(fold(s0, jnp.maximum), s1))

            mrun = jax.lax.fori_loop(
                0, nper, k_step, jnp.full((8, 128), -jnp.inf, f32))
            m = jnp.max(mrun, axis=-1, keepdims=True)

            def v_step(j, c):
                ls, acc = c
                issue_in_v_phase(n, j + AHEAD)

                @pl.when(both(last, j == 0))
                def _():
                    ob[...] = of[...].reshape(BH, D).astype(ob.dtype)
                    for cpy in early:
                        cpy.start()

                @pl.when(both(last, j == 1))
                def _():
                    pt = jnp.exp(sc[nper - 1, :, CA:] - m).T
                    for h in range(8):
                        wb[h] = jnp.broadcast_to(pt[:, sub[h]:sub[h] + 1], wb.shape[1:])

                p, ps = probs(j, m)
                xs = fetch(vbufs, j * BR, BR, j)
                return (ls + ps,
                        acc + pv(p[:, 0:CA], xs, part_a) + pv(p[:, CA:], xs, part_b))

            ls, acc = jax.lax.fori_loop(
                0, jnp.where(last, nper - 1, nper), v_step, (zero, zero))

            @pl.when(n != npair - 1)
            def _():
                res = acc / jnp.sum(ls, axis=-1, keepdims=True)
                for t, mask in zip(ts, row_masks):
                    of[t] = jnp.where(mask, res, of[t])

            return m, ls, acc

        m, ls, acc = jax.lax.fori_loop(
            0, npair, pair, (jnp.zeros((8, 1), f32), zero, zero))

        j = nper - 1
        p, ps = probs(j, m)
        rl = 1.0 / jnp.sum(ls + ps, axis=-1, keepdims=True)
        tiles = {t: of[t] for t in range(o_lo // 8, o_hi // 8)}
        for cpy in early:
            cpy.wait()
        acc = acc + pv(p[:, 0:CA], fetch(vbufs, j * BR, R1, j), part_a)

        def pv_vpu(r0, r1, si):
            c0, n = upH * (r0 - R1), upH * (r1 - r0)
            xs = fetch(vbufs, j * BR + r0, r1 - r0, si)
            return [jnp.sum((wb[h, c0:c0 + n] * part(xs, h, 0, r1 - r0).astype(f32))
                            .reshape(n // 8, 8, D), axis=0) for h in range(8)]

        first = pv_vpu(R1, R2, nper)
        acc = acc + pick([
            jnp.broadcast_to(jnp.sum(x + y, axis=0, keepdims=True), (8, D))
            for x, y in zip(first, pv_vpu(R2, BR, nper + 1))])
        res = acc * rl
        for t, mask in zip(last_tiles, row_masks):
            tiles[t] = jnp.where(mask, res, tiles[t])
        ob[o_lo:o_hi, :] = jnp.concatenate(
            [tiles[t] for t in sorted(tiles)], axis=0).astype(ob.dtype)
        late = pltpu.make_async_copy(
            ob.at[pl.ds(o_lo, o_hi - o_lo)], o_hbm.at[pl.ds(o_lo, o_hi - o_lo)],
            xsem.at[0])
        late.start()
        pltpu.make_async_copy(pace, pace, xsem.at[2]).wait()
        late.wait()

    out = pl.pallas_call(
        kern,
        in_specs=[pl.BlockSpec(memory_space=pl.ANY)] * 3,
        out_specs=pl.BlockSpec(memory_space=pl.ANY),
        out_shape=jax.ShapeDtypeStruct((BH, D), q.dtype),
        scratch_shapes=[
            pltpu.VMEM((G, U, D), k.dtype),
            pltpu.VMEM((G, U, D), k.dtype),
            pltpu.VMEM((G, U, D), v.dtype),
            pltpu.VMEM((G, U, D), v.dtype),
            pltpu.VMEM((LAG, CR, D), k.dtype),
            pltpu.SemaphoreType.DMA((2, nper + 2)),
            pltpu.SemaphoreType.DMA((3,)),
            pltpu.VMEM((nper, 8, upH * BR), f32),
            pltpu.VMEM((BH, D), q.dtype),
            pltpu.VMEM((BH // 8, 8, D), f32),
            pltpu.VMEM((BH // 8, 8, D), f32),
            pltpu.VMEM((BH, D), q.dtype),
            pltpu.VMEM((8, upH * (BR - R1), D), f32),
        ],
        compiler_params=pltpu.CompilerParams(
            vmem_limit_bytes=48 * 1024 * 1024,
            disable_bounds_checks=True, disable_semaphore_checks=True),
    )(q.reshape(BH, D), k.reshape(NU, U, D), v.reshape(NU, U, D))
    return out.reshape(B, H, Sq, D)
```
